```python
import jax
import jax.numpy as jnp

def _softmax(x, axis=-1):
    return jax.nn.softmax(x, axis=axis)
def _gelu(x):
    return jax.nn.gelu(x, approximate=True)
def _silu(x):
    return jax.nn.silu(x)
def _sigmoid(x):
    return jax.nn.sigmoid(x)
def _layernorm(x, axis=-1, eps=1e-5):
    m = jnp.mean(x, axis=axis, keepdims=True)
    v = jnp.var(x, axis=axis, keepdims=True)
    return (x - m) / jnp.sqrt(v + eps)
def _scatter_add(tgt, idx, src, axis=0):
    return tgt.at[idx].add(src)
def _segment_sum(src, seg, n):
    return jax.ops.segment_sum(src, seg, n)
class _Rng:
    def __init__(self, key):
        self._k = key
    def _next(self):
        self._k, sub = jax.random.split(self._k)
        return sub
    def normal(self, shape):
        return jax.random.normal(self._next(), shape, dtype=jnp.bfloat16)
    def randint(self, lo, hi, shape):
        return jax.random.randint(self._next(), shape, lo, hi, dtype=jnp.int32)
    def uniform(self, shape, lo=0.0, hi=1.0):
        return jax.random.uniform(self._next(), shape, jnp.bfloat16, lo, hi)
    def permutation(self, n):
        return jax.random.permutation(self._next(), n)


kernel_name = 'gated_mix__compressed_kv_cla__ssm_conv_s5__prompt'

def setup_inputs():
    _rng = _Rng(jax.random.key(int.from_bytes(__import__("os").urandom(4), "little")))
    _w = (lambda a: (lambda t: t.astype(jnp.bfloat16) if jnp.issubdtype(t.dtype, jnp.floating) else t)(jnp.asarray(a)))
    def _A_setup():
        B, H, Sq, Sk, D, M = 1, 16, 2048, 2048, 256, 448
        Dc = 4 * D
        return {
            "x": _w((lambda *s: _rng.normal(s) * 0.05)(B, Sq, M)),
            "c_kv": _w((lambda *s: _rng.normal(s) * 0.05)(B, Sk, Dc)),
            "w_q": _w((lambda *s: _rng.normal(s) * 0.05)(M, H, D) * (M ** -0.5)),
            "w_uk": _w((lambda *s: _rng.normal(s) * 0.05)(Dc, H, D) * (Dc ** -0.5)),
            "w_uv": _w((lambda *s: _rng.normal(s) * 0.05)(Dc, H, D) * (Dc ** -0.5)),
            "w_o": _w((lambda *s: _rng.normal(s) * 0.05)(H, D, M) * ((H * D) ** -0.5)),
        }
    _A_in = _A_setup()

    def _B_setup():
        B, S, D = 1, 2048, 448
        P = D
        Lambda_re = -0.5 * jnp.exp((lambda *s: _rng.normal(s) * 0.05)(P))
        Lambda_im = (lambda *s: _rng.normal(s) * 0.05)(P) * 1.0
        B_re = (lambda *s: _rng.normal(s) * 0.05)(P, D) * (D ** -0.5)
        B_im = (lambda *s: _rng.normal(s) * 0.05)(P, D) * (D ** -0.5)
        C_re = (lambda *s: _rng.normal(s) * 0.05)(D, P) * (P ** -0.5)
        C_im = (lambda *s: _rng.normal(s) * 0.05)(D, P) * (P ** -0.5)
        log_dt = (lambda *s: _rng.normal(s) * 0.05)(P) * 0.3 - 2.0
        Dskip = (lambda *s: _rng.normal(s) * 0.05)(D)
        return {
            "x": _w((lambda *s: _rng.normal(s) * 0.05)(B, S, D)),
            "Lambda_re": _w(Lambda_re),
            "Lambda_im": _w(Lambda_im),
            "B_re": _w(B_re),
            "B_im": _w(B_im),
            "C_re": _w(C_re),
            "C_im": _w(C_im),
            "log_dt": _w(log_dt),
            "Dskip": _w(Dskip),
        }
    _B_in = _B_setup()

    return {
        "A_x": _A_in["x"],
        "A_c_kv": _A_in["c_kv"],
        "A_w_q": _A_in["w_q"],
        "A_w_uk": _A_in["w_uk"],
        "A_w_uv": _A_in["w_uv"],
        "A_w_o": _A_in["w_o"],
        "B_x": _B_in["x"],
        "B_Lambda_re": _B_in["Lambda_re"],
        "B_Lambda_im": _B_in["Lambda_im"],
        "B_B_re": _B_in["B_re"],
        "B_B_im": _B_in["B_im"],
        "B_C_re": _B_in["C_re"],
        "B_C_im": _B_in["C_im"],
        "B_log_dt": _B_in["log_dt"],
        "B_Dskip": _B_in["Dskip"],
        "gate_w": _w((lambda *s: _rng.normal(s) * 0.05)(448)),
    }

def reference(A_x, A_c_kv, A_w_q, A_w_uk, A_w_uv, A_w_o, B_x, B_Lambda_re, B_Lambda_im, B_B_re, B_B_im, B_C_re, B_C_im, B_log_dt, B_Dskip, gate_w):
    def _A_ref(x, c_kv, w_q, w_uk, w_uv, w_o):
        B, Sq, M = x.shape[0], x.shape[1], x.shape[2]
        Sk = c_kv.shape[1]
        H, D = w_q.shape[1], w_q.shape[2]
        q = jnp.einsum("bqm,mhd->bhqd", x, w_q)
        k = jnp.einsum("bkc,chd->bhkd", c_kv, w_uk)
        v = jnp.einsum("bkc,chd->bhkd", c_kv, w_uv)
        scores = jnp.einsum("bhqd,bhkd->bhqk", q, k) * (D ** -0.5)
        off = Sk - Sq
        qi = jnp.arange(Sq)[:, None]
        kj = jnp.arange(Sk)[None, :]
        cmask = kj <= (qi + off)
        scores = jnp.where(cmask[None, None], scores, -1e9)
        p = _softmax(scores, axis=-1)
        ctx = jnp.einsum("bhqk,bhkd->bhqd", p, v)
        return jnp.einsum("bhqd,hdm->bqm", ctx, w_o)

    def _B_ref(x, Lambda_re, Lambda_im, B_re, B_im, C_re, C_im, log_dt, Dskip):
        Bsz, L, H = x.shape
        Lam = Lambda_re + 1j * Lambda_im
        Bmat = B_re + 1j * B_im
        Cmat = C_re + 1j * C_im
        dt = jnp.exp(log_dt)
        Lam_bar = jnp.exp(dt * Lam)
        B_bar = ((Lam_bar - 1.0) / Lam)[:, None] * Bmat
        Bu = jnp.einsum("bld,pd->blp", x + 0j, B_bar)
        h = jnp.zeros_like(Bu[:, 0, :])
        hs = []
        for t in range(L):
            h = Lam_bar[None, :] * h + Bu[:, t, :]
            hs.append(h)
        hseq = jnp.stack(hs, 1)
        y = 2.0 * jnp.einsum("blp,dp->bld", hseq, Cmat).real + x * Dskip[None, None, :]
        return y

    x = A_x
    g = _sigmoid((x * gate_w).sum(-1, keepdims=True))
    a = _A_ref(x, A_c_kv, A_w_q, A_w_uk, A_w_uv, A_w_o)
    b = _B_ref(x, B_Lambda_re, B_Lambda_im, B_B_re, B_B_im, B_C_re, B_C_im, B_log_dt, B_Dskip)
    return g * a + (1 - g) * b
```

```python
import functools
import math

import jax
import jax.numpy as jnp
import jax.experimental.pallas as pl
import jax.experimental.pallas.tpu as pltpu

F32 = jnp.float32
BF16 = jnp.bfloat16
NN = (((1,), (0,)), ((), ()))
NT = (((1,), (1,)), ((), ()))


def _dot(a, b, dims=NN):
    return jax.lax.dot_general(a, b, dims, preferred_element_type=F32)


def _unpack(u):
    lo = pltpu.bitcast(u << 16, F32).astype(BF16)
    hi = pltpu.bitcast(u & jnp.uint32(0xFFFF0000), F32).astype(BF16)
    return lo, hi


def _cmul(ar, ai, br, bi):
    return ar * br - ai * bi, ar * bi + ai * br


def _kernel(xT_hbm, ckv_hbm, wq_hbm, wuk_hbm, wuv_hbm, woT_hbm,
            lre_ref, lim_ref, bre_hbm, bim_hbm, cre_hbm, cim_hbm, ldt_ref, dsk_ref, gw_ref,
            out_hbm,
            xT, ckv, wq32, wuk32, wuv32, woT, bre, bim, cre, cim,
            qT, kk, vT, ctxT, s_buf, ur, ui, hr, hi_, coef, obuf,
            sem_in, sem_w, sem_out, *, S, M, H, D, C, BQ, BT):
    NP = H // 2
    wq_u = wq_hbm.bitcast(jnp.uint32)
    wuk_u = wuk_hbm.bitcast(jnp.uint32)
    wuv_u = wuv_hbm.bitcast(jnp.uint32)

    def w_copies(j, slot):
        return (pltpu.make_async_copy(wq_u.at[:, j, :], wq32.at[slot], sem_w.at[0, slot]),
                pltpu.make_async_copy(wuk_u.at[:, j, :], wuk32.at[slot], sem_w.at[1, slot]),
                pltpu.make_async_copy(wuv_u.at[:, j, :], wuv32.at[slot], sem_w.at[2, slot]))

    cp_x = pltpu.make_async_copy(xT_hbm, xT, sem_in.at[0])
    cp_c = pltpu.make_async_copy(ckv_hbm, ckv, sem_in.at[1])
    late = [pltpu.make_async_copy(s, d, sem_in.at[2 + i]) for i, (s, d) in enumerate(
        [(woT_hbm, woT), (bre_hbm, bre), (bim_hbm, bim), (cre_hbm, cre), (cim_hbm, cim)])]

    w0 = w_copies(0, 0)
    cp_x.start()
    w0[0].start()
    cp_c.start()
    w0[1].start()
    w0[2].start()

    scale = (D ** -0.5) * math.log2(math.e)
    neg = -1e30

    def pair_body(j, carry):
        slot = j % 2
        cq, ck, cv = w_copies(j, slot)

        @pl.when(j == 0)
        def _():
            cp_x.wait()

        cq.wait()
        lo, hi = _unpack(wq32[slot].T)
        wqT = jnp.concatenate([lo, hi], axis=0)
        qT[...] = (_dot(wqT, xT[...]) * scale).astype(BF16)

        @pl.when(j == 0)
        def _():
            cp_c.wait()

        ck.wait()
        cv.wait()

        @pl.when(j + 1 < NP)
        def _():
            for c in w_copies(j + 1, 1 - slot):
                c.start()

        @pl.when(j == 0)
        def _():
            for c in late:
                c.start()

        lo, hi = _unpack(wuk32[slot])
        kp = _dot(ckv[...], jnp.concatenate([lo, hi], axis=1)).astype(BF16)
        kk[0] = kp[:, :D]
        kk[1] = kp[:, D:]
        lo, hi = _unpack(wuv32[slot].T)
        vT[...] = _dot(jnp.concatenate([lo, hi], axis=0), ckv[...], NT).astype(BF16)

        def head_body(e, carry2):
            r = pl.ds(pl.multiple_of(e * D, D), D)
            ro = pl.ds(pl.multiple_of((2 * j + e) * D, D), D)
            for i in range(S // BQ):
                L = (i + 1) * BQ
                q = qT[r, i * BQ:(i + 1) * BQ]
                row = jax.lax.broadcasted_iota(jnp.int32, (BQ, BQ), 0)
                col = jax.lax.broadcasted_iota(jnp.int32, (BQ, BQ), 1)
                sd = _dot(kk[e, i * BQ:L, :], q)
                sd = jnp.where(row <= col, sd, neg)
                m = jnp.max(sd, axis=0, keepdims=True)
                if i > 0:
                    so = _dot(kk[e, 0:i * BQ, :], q)
                    m = jnp.maximum(m, jnp.max(so, axis=0, keepdims=True))
                    po = jnp.exp2(so - m)
                pd = jnp.exp2(sd - m)
                l = jnp.sum(pd, axis=0, keepdims=True)
                o = _dot(vT[r, i * BQ:L], pd.astype(BF16))
                if i > 0:
                    l = l + jnp.sum(po, axis=0, keepdims=True)
                    o = o + _dot(vT[r, 0:i * BQ], po.astype(BF16))
                ctxT[ro, i * BQ:(i + 1) * BQ] = (o * (1.0 / l)).astype(BF16)
            return carry2

        jax.lax.fori_loop(0, 2, head_body, 0)
        return carry

    jax.lax.fori_loop(0, NP, pair_body, 0)

    for c in late:
        c.wait()

    lre = lre_ref[...].astype(F32).reshape(1, M)
    lim = lim_ref[...].astype(F32).reshape(1, M)
    dt = jnp.exp(ldt_ref[...].astype(F32)).astype(BF16).astype(F32).reshape(1, M)
    mag = jnp.exp(dt * lre)
    ar, ai = mag * jnp.cos(dt * lim), mag * jnp.sin(dt * lim)
    den = lre * lre + lim * lim
    zr, zi = _cmul(ar - 1.0, ai, lre / den, -lim / den)
    p1 = (ar, ai)
    p2 = _cmul(*p1, *p1)
    p4 = _cmul(*p2, *p2)
    rid = jax.lax.broadcasted_iota(jnp.int32, (8, M), 0)
    for n, (k, (pr, pi)) in enumerate(((1, p1), (2, p2), (4, p4))):
        coef[2 * n] = jnp.where(rid >= k, pr, 0.0)
        coef[2 * n + 1] = jnp.where(rid >= k, pi, 0.0)
    cr, ci = jnp.broadcast_to(ar, (8, M)), jnp.broadcast_to(ai, (8, M))
    pw = p1
    for t in range(1, 8):
        pw = _cmul(*pw, *p1)
        cr = jnp.where(rid == t, pw[0], cr)
        ci = jnp.where(rid == t, pw[1], ci)
    coef[6] = cr
    coef[7] = ci
    czr, czi = _cmul(cre[...].astype(F32), cim[...].astype(F32), 2.0 * zr, 2.0 * zi)
    cre[...] = czr.astype(BF16)
    cim[...] = (-czi).astype(BF16)
    gcol = jnp.broadcast_to(gw_ref[...].astype(F32).reshape(1, M), (128, M)).T
    dcol = jnp.broadcast_to(dsk_ref[...].astype(F32).reshape(1, M), (128, M)).T

    def out_copy(i, slot):
        return pltpu.make_async_copy(
            obuf.at[slot], out_hbm.at[:, pl.ds(pl.multiple_of(i * BT, BT), BT)], sem_out.at[slot])

    def out_body(i, carry):
        car, cai = carry
        c = pl.ds(pl.multiple_of(i * BT, BT), BT)
        slot = i % 2
        bx = xT[:, c]
        bxt = bx.T
        ur[...] = _dot(bxt, bre[...], NT)
        ui[...] = _dot(bxt, bim[...], NT)
        for g in range(BT // 8):
            a, b = ur[g * 8:(g + 1) * 8, :], ui[g * 8:(g + 1) * 8, :]
            for n, k in enumerate((1, 2, 4)):
                dr, di = _cmul(coef[2 * n], coef[2 * n + 1], pltpu.roll(a, k, 0), pltpu.roll(b, k, 0))
                a, b = a + dr, b + di
            dr, di = _cmul(coef[6], coef[7], car, cai)
            a, b = a + dr, b + di
            car = jnp.broadcast_to(a[7:8, :], (8, M))
            cai = jnp.broadcast_to(b[7:8, :], (8, M))
            hr[g * 8:(g + 1) * 8, :] = a
            hi_[g * 8:(g + 1) * 8, :] = b
        att = _dot(woT[0], ctxT[0:D, c])
        for h in range(1, H):
            att = att + _dot(woT[h], ctxT[h * D:(h + 1) * D, c])
        y = _dot(cre[...], hr[...].astype(BF16), NT) + _dot(cim[...], hi_[...].astype(BF16), NT)
        rep = BT // 128
        y = y + bx.astype(F32) * jnp.tile(dcol, (1, rep))
        z = jnp.sum(bx.astype(F32) * jnp.tile(gcol, (1, rep)), axis=0, keepdims=True)
        gate = 1.0 / (1.0 + jnp.exp(-z))

        @pl.when(i >= 2)
        def _():
            out_copy(i - 2, slot).wait()

        obuf[slot] = gate * att + (1.0 - gate) * y
        out_copy(i, slot).start()
        return car, cai

    zero = jnp.zeros((8, M), F32)
    nb = S // BT
    jax.lax.fori_loop(0, nb, out_body, (zero, zero))
    out_copy(nb - 2, (nb - 2) % 2).wait()
    out_copy(nb - 1, (nb - 1) % 2).wait()


@jax.jit
def pallas_gated_mix__compressed_kv_cla__ssm_conv_s5__prompt_kernel(
    A_x, A_c_kv, A_w_q, A_w_uk, A_w_uv, A_w_o, B_x, B_Lambda_re, B_Lambda_im,
    B_B_re, B_B_im, B_C_re, B_C_im, B_log_dt, B_Dskip, gate_w,
):
    _, S, M = A_x.shape
    C = A_c_kv.shape[2]
    H, D = A_w_q.shape[1], A_w_q.shape[2]
    BQ, BT = 256, 512
    hbm = pl.BlockSpec(memory_space=pl.ANY)
    vm = pl.BlockSpec(memory_space=pltpu.VMEM)
    V = pltpu.VMEM
    outT = pl.pallas_call(
        functools.partial(_kernel, S=S, M=M, H=H, D=D, C=C, BQ=BQ, BT=BT),
        out_shape=jax.ShapeDtypeStruct((M, S), F32),
        in_specs=[hbm] * 6 + [vm, vm] + [hbm] * 4 + [vm, vm, vm],
        out_specs=hbm,
        scratch_shapes=[
            V((M, S), BF16), V((S, C), BF16),
            V((2, M, D), jnp.uint32), V((2, C, D), jnp.uint32), V((2, C, D), jnp.uint32),
            V((H, M, D), BF16),
            V((M, M), BF16), V((M, M), BF16), V((M, M), BF16), V((M, M), BF16),
            V((2 * D, S), BF16), V((2, S, D), BF16), V((2 * D, S), BF16), V((H * D, S), BF16),
            V((S, BQ), F32), V((BT, M), F32), V((BT, M), F32), V((BT, M), F32), V((BT, M), F32),
            V((8, 8, M), F32), V((2, M, BT), F32),
            pltpu.SemaphoreType.DMA((8,)), pltpu.SemaphoreType.DMA((3, 2)), pltpu.SemaphoreType.DMA((2,)),
        ],
        compiler_params=pltpu.CompilerParams(vmem_limit_bytes=110 * 1024 * 1024),
    )(A_x[0].T, A_c_kv[0], A_w_q, A_w_uk, A_w_uv, A_w_o.transpose(0, 2, 1),
      B_Lambda_re, B_Lambda_im, B_B_re, B_B_im, B_C_re, B_C_im, B_log_dt, B_Dskip, gate_w)
    return outT.T[None]
```

```python
import functools
import math

import jax
import jax.numpy as jnp
import jax.experimental.pallas as pl
import jax.experimental.pallas.tpu as pltpu

F32 = jnp.float32
BF16 = jnp.bfloat16
NN = (((1,), (0,)), ((), ()))
NT = (((1,), (1,)), ((), ()))


def _dot(a, b, dims=NN):
    return jax.lax.dot_general(a, b, dims, preferred_element_type=F32)


def _unpack(u):
    lo = pltpu.bitcast(u << 16, F32).astype(BF16)
    hi = pltpu.bitcast(u & jnp.uint32(0xFFFF0000), F32).astype(BF16)
    return lo, hi


def _cmul(ar, ai, br, bi):
    return ar * br - ai * bi, ar * bi + ai * br


def _kernel(xT_hbm, ckv_hbm, wq_hbm, wuk_hbm, wuv_hbm, woT_hbm,
            lre_ref, lim_ref, bre_hbm, bim_hbm, cre_hbm, cim_hbm, ldt_ref, dsk_ref, gw_ref,
            out_hbm,
            xT, ckv, wq32, wuk32, wuv32, woT, bre, bim, cre, cim,
            qT, kk, vT, ctxT, s_buf, ur, ui, hr, hi_, coef, obuf,
            sem_in, sem_w, sem_out, *, S, M, H, D, C, BQ, BT):
    NP = H // 2
    wq_u = wq_hbm.bitcast(jnp.uint32)
    wuk_u = wuk_hbm.bitcast(jnp.uint32)
    wuv_u = wuv_hbm.bitcast(jnp.uint32)

    def w_copies(j, slot):
        return (pltpu.make_async_copy(wq_u.at[:, j, :], wq32.at[slot], sem_w.at[0, slot]),
                pltpu.make_async_copy(wuk_u.at[:, j, :], wuk32.at[slot], sem_w.at[1, slot]),
                pltpu.make_async_copy(wuv_u.at[:, j, :], wuv32.at[slot], sem_w.at[2, slot]))

    cp_x = pltpu.make_async_copy(xT_hbm, xT, sem_in.at[0])
    cp_c = pltpu.make_async_copy(ckv_hbm, ckv, sem_in.at[1])
    late = [pltpu.make_async_copy(s, d, sem_in.at[2 + i]) for i, (s, d) in enumerate(
        [(woT_hbm, woT), (bre_hbm, bre), (bim_hbm, bim), (cre_hbm, cre), (cim_hbm, cim)])]

    w0 = w_copies(0, 0)
    cp_x.start()
    w0[0].start()
    cp_c.start()
    w0[1].start()
    w0[2].start()

    scale = (D ** -0.5) * math.log2(math.e)
    neg = -1e30

    def pair_body(j, carry):
        slot = j % 2
        cq, ck, cv = w_copies(j, slot)

        @pl.when(j == 0)
        def _():
            cp_x.wait()

        cq.wait()
        lo, hi = _unpack(wq32[slot].T)
        wqT = jnp.concatenate([lo, hi], axis=0)
        qT[...] = (_dot(wqT, xT[...]) * scale).astype(BF16)

        @pl.when(j == 0)
        def _():
            cp_c.wait()

        ck.wait()
        cv.wait()

        @pl.when(j + 1 < NP)
        def _():
            for c in w_copies(j + 1, 1 - slot):
                c.start()

        @pl.when(j == 0)
        def _():
            for c in late:
                c.start()

        lo, hi = _unpack(wuk32[slot])
        kp = _dot(ckv[...], jnp.concatenate([lo, hi], axis=1)).astype(BF16)
        kk[0] = kp[:, :D]
        kk[1] = kp[:, D:]
        lo, hi = _unpack(wuv32[slot].T)
        vT[...] = _dot(jnp.concatenate([lo, hi], axis=0), ckv[...], NT).astype(BF16)

        def head_body(e, carry2):
            r = pl.ds(pl.multiple_of(e * D, D), D)
            ro = pl.ds(pl.multiple_of((2 * j + e) * D, D), D)
            nq = S // BQ
            T = BQ // 2
            row = jax.lax.broadcasted_iota(jnp.int32, (T, T), 0)
            col = jax.lax.broadcasted_iota(jnp.int32, (T, T), 1)
            tri = row <= col

            def scores(i):
                L = i * BQ + T
                q = qT[r, i * BQ:(i + 1) * BQ]
                s = _dot(kk[e, 0:L, :], q)
                sx = jnp.where(tri, _dot(kk[e, L:L + T, :], q[:, T:]), neg)
                sd = jnp.concatenate([jnp.where(tri, s[L - T:, :T], neg), s[L - T:, T:]], axis=1)
                if i > 0:
                    sd = jnp.concatenate([s[:L - T], sd], axis=0)
                m = jnp.max(sd, axis=0, keepdims=True)
                m = jnp.concatenate([m[:, :T], jnp.maximum(m[:, T:], jnp.max(sx, axis=0, keepdims=True))], axis=1)
                return sd, sx, m

            nxt = scores(0)
            for i in range(nq):
                s, sx, m = nxt
                if i + 1 < nq:
                    nxt = scores(i + 1)
                L = i * BQ + T
                p = jnp.exp2(s - m)
                px = jnp.exp2(sx - m[:, T:])
                l = jnp.sum(p, axis=0, keepdims=True)
                o = _dot(vT[r, 0:L], p.astype(BF16))
                ox = _dot(vT[r, L:L + T], px.astype(BF16))
                la = 1.0 / l[:, :T]
                lb = 1.0 / (l[:, T:] + jnp.sum(px, axis=0, keepdims=True))
                ctxT[ro, i * BQ:L] = (o[:, :T] * la).astype(BF16)
                ctxT[ro, L:L + T] = ((o[:, T:] + ox) * lb).astype(BF16)
            return carry2

        jax.lax.fori_loop(0, 2, head_body, 0)
        return carry

    jax.lax.fori_loop(0, NP, pair_body, 0)

    for c in late:
        c.wait()

    lre = lre_ref[...].astype(F32).reshape(1, M)
    lim = lim_ref[...].astype(F32).reshape(1, M)
    dt = jnp.exp(ldt_ref[...].astype(F32)).astype(BF16).astype(F32).reshape(1, M)
    mag = jnp.exp(dt * lre)
    ar, ai = mag * jnp.cos(dt * lim), mag * jnp.sin(dt * lim)
    den = lre * lre + lim * lim
    zr, zi = _cmul(ar - 1.0, ai, lre / den, -lim / den)
    p1 = (ar, ai)
    p2 = _cmul(*p1, *p1)
    p4 = _cmul(*p2, *p2)
    rid = jax.lax.broadcasted_iota(jnp.int32, (8, M), 0)
    for n, (k, (pr, pi)) in enumerate(((1, p1), (2, p2), (4, p4))):
        coef[2 * n] = jnp.where(rid >= k, pr, 0.0)
        coef[2 * n + 1] = jnp.where(rid >= k, pi, 0.0)
    cr, ci = jnp.broadcast_to(ar, (8, M)), jnp.broadcast_to(ai, (8, M))
    pw = p1
    for t in range(1, 8):
        pw = _cmul(*pw, *p1)
        cr = jnp.where(rid == t, pw[0], cr)
        ci = jnp.where(rid == t, pw[1], ci)
    coef[6] = cr
    coef[7] = ci
    czr, czi = _cmul(cre[...].astype(F32), cim[...].astype(F32), 2.0 * zr, 2.0 * zi)
    cre[...] = czr.astype(BF16)
    cim[...] = (-czi).astype(BF16)
    gcol = jnp.broadcast_to(gw_ref[...].astype(F32).reshape(1, M), (128, M)).T
    dcol = jnp.broadcast_to(dsk_ref[...].astype(F32).reshape(1, M), (128, M)).T

    def out_copy(i, slot):
        return pltpu.make_async_copy(
            obuf.at[slot], out_hbm.at[:, pl.ds(pl.multiple_of(i * BT, BT), BT)], sem_out.at[slot])

    def out_body(i, carry):
        car, cai = carry
        c = pl.ds(pl.multiple_of(i * BT, BT), BT)
        slot = i % 2
        bx = xT[:, c]
        bxt = bx.T
        ur[...] = _dot(bxt, bre[...], NT)
        ui[...] = _dot(bxt, bim[...], NT)
        for g in range(BT // 8):
            a, b = ur[g * 8:(g + 1) * 8, :], ui[g * 8:(g + 1) * 8, :]
            for n, k in enumerate((1, 2, 4)):
                dr, di = _cmul(coef[2 * n], coef[2 * n + 1], pltpu.roll(a, k, 0), pltpu.roll(b, k, 0))
                a, b = a + dr, b + di
            dr, di = _cmul(coef[6], coef[7], car, cai)
            a, b = a + dr, b + di
            car = jnp.broadcast_to(a[7:8, :], (8, M))
            cai = jnp.broadcast_to(b[7:8, :], (8, M))
            hr[g * 8:(g + 1) * 8, :] = a
            hi_[g * 8:(g + 1) * 8, :] = b
        att = _dot(woT[0], ctxT[0:D, c])
        for h in range(1, H):
            att = att + _dot(woT[h], ctxT[h * D:(h + 1) * D, c])
        y = _dot(cre[...], hr[...].astype(BF16), NT) + _dot(cim[...], hi_[...].astype(BF16), NT)
        rep = BT // 128
        y = y + bx.astype(F32) * jnp.tile(dcol, (1, rep))
        z = jnp.sum(bx.astype(F32) * jnp.tile(gcol, (1, rep)), axis=0, keepdims=True)
        gate = 1.0 / (1.0 + jnp.exp(-z))

        @pl.when(i >= 2)
        def _():
            out_copy(i - 2, slot).wait()

        obuf[slot] = gate * att + (1.0 - gate) * y
        out_copy(i, slot).start()
        return car, cai

    zero = jnp.zeros((8, M), F32)
    nb = S // BT
    jax.lax.fori_loop(0, nb, out_body, (zero, zero))
    out_copy(nb - 2, (nb - 2) % 2).wait()
    out_copy(nb - 1, (nb - 1) % 2).wait()


@jax.jit
def pallas_gated_mix__compressed_kv_cla__ssm_conv_s5__prompt_kernel(
    A_x, A_c_kv, A_w_q, A_w_uk, A_w_uv, A_w_o, B_x, B_Lambda_re, B_Lambda_im,
    B_B_re, B_B_im, B_C_re, B_C_im, B_log_dt, B_Dskip, gate_w,
):
    _, S, M = A_x.shape
    C = A_c_kv.shape[2]
    H, D = A_w_q.shape[1], A_w_q.shape[2]
    BQ, BT = 256, 512
    hbm = pl.BlockSpec(memory_space=pl.ANY)
    vm = pl.BlockSpec(memory_space=pltpu.VMEM)
    V = pltpu.VMEM
    outT = pl.pallas_call(
        functools.partial(_kernel, S=S, M=M, H=H, D=D, C=C, BQ=BQ, BT=BT),
        out_shape=jax.ShapeDtypeStruct((M, S), F32),
        in_specs=[hbm] * 6 + [vm, vm] + [hbm] * 4 + [vm, vm, vm],
        out_specs=hbm,
        scratch_shapes=[
            V((M, S), BF16), V((S, C), BF16),
            V((2, M, D), jnp.uint32), V((2, C, D), jnp.uint32), V((2, C, D), jnp.uint32),
            V((H, M, D), BF16),
            V((M, M), BF16), V((M, M), BF16), V((M, M), BF16), V((M, M), BF16),
            V((2 * D, S), BF16), V((2, S, D), BF16), V((2 * D, S), BF16), V((H * D, S), BF16),
            V((S, BQ), F32), V((BT, M), F32), V((BT, M), F32), V((BT, M), F32), V((BT, M), F32),
            V((8, 8, M), F32), V((2, M, BT), F32),
            pltpu.SemaphoreType.DMA((8,)), pltpu.SemaphoreType.DMA((3, 2)), pltpu.SemaphoreType.DMA((2,)),
        ],
        compiler_params=pltpu.CompilerParams(vmem_limit_bytes=110*1024*1024, flags={"XLA_TPU_FORCE_LP_LLO_SCHEDULER": True}),
    )(A_x[0].T, A_c_kv[0], A_w_q, A_w_uk, A_w_uv, A_w_o.transpose(0, 2, 1),
      B_Lambda_re, B_Lambda_im, B_B_re, B_B_im, B_C_re, B_C_im, B_log_dt, B_Dskip, gate_w)
    return outT.T[None]
```

```python
import functools
import math

import jax
import jax.numpy as jnp
import jax.experimental.pallas as pl
import jax.experimental.pallas.tpu as pltpu

F32 = jnp.float32
BF16 = jnp.bfloat16
NN = (((1,), (0,)), ((), ()))
NT = (((1,), (1,)), ((), ()))


def _dot(a, b, dims=NN):
    return jax.lax.dot_general(a, b, dims, preferred_element_type=F32)


def _unpack(u):
    lo = pltpu.bitcast(u << 16, F32).astype(BF16)
    hi = pltpu.bitcast(u & jnp.uint32(0xFFFF0000), F32).astype(BF16)
    return lo, hi


def _cmul(ar, ai, br, bi):
    return ar * br - ai * bi, ar * bi + ai * br


def _kernel(xT_hbm, ckv_hbm, wq_hbm, wuk_hbm, wuv_hbm, woT_hbm,
            lre_ref, lim_ref, bre_hbm, bim_hbm, cre_hbm, cim_hbm, ldt_ref, dsk_ref, gw_ref,
            out_hbm,
            xT, ckv, wq32, wuk32, wuv32, woT, bre, bim, cre, cim,
            qT, kk, vT, ctxT, ur, ui, hr, hi_, coef, obuf,
            sem_in, sem_x, sem_w, sem_out, *, S, M, H, D, C, BQ, BT, BU):
    NP = H // 2
    wq_u = wq_hbm.bitcast(jnp.uint32)
    wuk_u = wuk_hbm.bitcast(jnp.uint32)
    wuv_u = wuv_hbm.bitcast(jnp.uint32)

    def w_copies(j, slot):
        return (pltpu.make_async_copy(wq_u.at[:, j, :], wq32.at[slot], sem_w.at[0, slot]),
                pltpu.make_async_copy(wuk_u.at[:, j, :], wuk32.at[slot], sem_w.at[1, slot]),
                pltpu.make_async_copy(wuv_u.at[:, j, :], wuv32.at[slot], sem_w.at[2, slot]))

    def x_copy(i):
        c = pl.ds(pl.multiple_of(i * BU, BU), BU)
        return pltpu.make_async_copy(xT_hbm.at[:, c], xT.at[:, c], sem_x.at[i])

    cp_c, cp_br, cp_bi, *late = [pltpu.make_async_copy(s, d, sem_in.at[i]) for i, (s, d) in enumerate(
        [(ckv_hbm, ckv), (bre_hbm, bre), (bim_hbm, bim), (woT_hbm, woT), (cre_hbm, cre), (cim_hbm, cim)])]

    cp_br.start()
    cp_bi.start()
    x_copy(0).start()

    lre = lre_ref[...].astype(F32).reshape(1, M)
    lim = lim_ref[...].astype(F32).reshape(1, M)
    dt = jnp.exp(ldt_ref[...].astype(F32)).astype(BF16).astype(F32).reshape(1, M)
    mag = jnp.exp(dt * lre)
    ar, ai = mag * jnp.cos(dt * lim), mag * jnp.sin(dt * lim)
    den = lre * lre + lim * lim
    zr, zi = _cmul(ar - 1.0, ai, lre / den, -lim / den)
    p1 = (ar, ai)
    p2 = _cmul(*p1, *p1)
    p4 = _cmul(*p2, *p2)
    rid = jax.lax.broadcasted_iota(jnp.int32, (8, M), 0)
    for n, (k, (pr, pi)) in enumerate(((1, p1), (2, p2), (4, p4))):
        coef[2 * n] = jnp.where(rid >= k, pr, 0.0)
        coef[2 * n + 1] = jnp.where(rid >= k, pi, 0.0)
    coef[6] = jnp.where(rid == 0, ar, 0.0)
    coef[7] = jnp.where(rid == 0, ai, 0.0)

    cp_br.wait()
    cp_bi.wait()
    for i in range(1, S // BU):
        x_copy(i).start()
    cp_c.start()
    for c in w_copies(0, 0):
        c.start()

    def bu_body(i, carry):
        c = pl.ds(pl.multiple_of(i * BU, BU), BU)
        x_copy(i).wait()
        x = xT[:, c].T
        a, b = _cmul(_dot(x, bre[...], NT), _dot(x, bim[...], NT), 2.0 * zr, 2.0 * zi)
        ur[c, :] = a
        ui[c, :] = b
        return carry

    jax.lax.fori_loop(0, S // BU, bu_body, 0)
    cp_c.wait()

    scale = (D ** -0.5) * math.log2(math.e)
    neg = -1e30

    def pair_body(j, carry):
        slot = j % 2
        cq, ck, cv = w_copies(j, slot)

        cq.wait()
        ck.wait()
        cv.wait()

        @pl.when(j + 1 < NP)
        def _():
            for c in w_copies(j + 1, 1 - slot):
                c.start()

        @pl.when(j == 0)
        def _():
            for c in late:
                c.start()

        lo, hi = _unpack(wq32[slot].T)
        wqT = jnp.concatenate([lo, hi], axis=0)
        qT[...] = (_dot(wqT, xT[...]) * scale).astype(BF16)

        lo, hi = _unpack(wuk32[slot])
        kp = _dot(ckv[...], jnp.concatenate([lo, hi], axis=1)).astype(BF16)
        kk[0] = kp[:, :D]
        kk[1] = kp[:, D:]
        lo, hi = _unpack(wuv32[slot].T)
        vT[...] = _dot(jnp.concatenate([lo, hi], axis=0), ckv[...], NT).astype(BF16)

        def head_body(e, carry2):
            r = pl.ds(pl.multiple_of(e * D, D), D)
            ro = pl.ds(pl.multiple_of((2 * j + e) * D, D), D)
            nq = S // BQ
            T = BQ // 2
            row = jax.lax.broadcasted_iota(jnp.int32, (T, T), 0)
            col = jax.lax.broadcasted_iota(jnp.int32, (T, T), 1)
            tri = row <= col

            def scores(i):
                L = i * BQ + T
                q = qT[r, i * BQ:(i + 1) * BQ]
                s = _dot(kk[e, 0:L, :], q)
                sx = jnp.where(tri, _dot(kk[e, L:L + T, :], q[:, T:]), neg)
                sd = jnp.concatenate([jnp.where(tri, s[L - T:, :T], neg), s[L - T:, T:]], axis=1)
                if i > 0:
                    sd = jnp.concatenate([s[:L - T], sd], axis=0)
                m = jnp.max(sd, axis=0, keepdims=True)
                m = jnp.concatenate([m[:, :T], jnp.maximum(m[:, T:], jnp.max(sx, axis=0, keepdims=True))], axis=1)
                return sd, sx, m

            nxt = scores(0)
            for i in range(nq):
                s, sx, m = nxt
                if i + 1 < nq:
                    nxt = scores(i + 1)
                L = i * BQ + T
                p = jnp.exp2(s - m)
                px = jnp.exp2(sx - m[:, T:])
                l = jnp.sum(p, axis=0, keepdims=True)
                o = _dot(vT[r, 0:L], p.astype(BF16))
                ox = _dot(vT[r, L:L + T], px.astype(BF16))
                la = 1.0 / l[:, :T]
                lb = 1.0 / (l[:, T:] + jnp.sum(px, axis=0, keepdims=True))
                ctxT[ro, i * BQ:L] = (o[:, :T] * la).astype(BF16)
                ctxT[ro, L:L + T] = ((o[:, T:] + ox) * lb).astype(BF16)
            return carry2

        jax.lax.fori_loop(0, 2, head_body, 0)
        return carry

    jax.lax.fori_loop(0, NP, pair_body, 0)

    for c in late:
        c.wait()

    gcol = jnp.broadcast_to(gw_ref[...].astype(F32).reshape(1, M), (128, M)).T
    dcol = jnp.broadcast_to(dsk_ref[...].astype(F32).reshape(1, M), (128, M)).T

    def out_copy(i, slot):
        return pltpu.make_async_copy(
            obuf.at[slot], out_hbm.at[:, pl.ds(pl.multiple_of(i * BT, BT), BT)], sem_out.at[slot])

    def out_body(i, carry):
        car, cai = carry
        c = pl.ds(pl.multiple_of(i * BT, BT), BT)
        slot = i % 2
        bx = xT[:, c]
        for g in range(BT // 8):
            t = pl.ds(pl.multiple_of(i * BT + g * 8, 8), 8)
            dr, di = _cmul(coef[6], coef[7], pltpu.roll(car, 1, 0), pltpu.roll(cai, 1, 0))
            a, b = ur[t, :] + dr, ui[t, :] + di
            for n, k in enumerate((1, 2, 4)):
                dr, di = _cmul(coef[2 * n], coef[2 * n + 1], pltpu.roll(a, k, 0), pltpu.roll(b, k, 0))
                a, b = a + dr, b + di
            car, cai = a, b
            hr[g * 8:(g + 1) * 8, :] = a
            hi_[g * 8:(g + 1) * 8, :] = b
        att = _dot(woT[0], ctxT[0:D, c])
        for h in range(1, H):
            att = att + _dot(woT[h], ctxT[h * D:(h + 1) * D, c])
        y = _dot(cre[...], hr[...].astype(BF16), NT) - _dot(cim[...], hi_[...].astype(BF16), NT)
        rep = BT // 128
        y = y + bx.astype(F32) * jnp.tile(dcol, (1, rep))
        z = jnp.sum(bx.astype(F32) * jnp.tile(gcol, (1, rep)), axis=0, keepdims=True)
        gate = 1.0 / (1.0 + jnp.exp(-z))

        @pl.when(i >= 2)
        def _():
            out_copy(i - 2, slot).wait()

        obuf[slot] = gate * att + (1.0 - gate) * y
        out_copy(i, slot).start()
        return car, cai

    zero = jnp.zeros((8, M), F32)
    nb = S // BT
    jax.lax.fori_loop(0, nb, out_body, (zero, zero))
    out_copy(nb - 2, (nb - 2) % 2).wait()
    out_copy(nb - 1, (nb - 1) % 2).wait()


@jax.jit
def pallas_gated_mix__compressed_kv_cla__ssm_conv_s5__prompt_kernel(
    A_x, A_c_kv, A_w_q, A_w_uk, A_w_uv, A_w_o, B_x, B_Lambda_re, B_Lambda_im,
    B_B_re, B_B_im, B_C_re, B_C_im, B_log_dt, B_Dskip, gate_w,
):
    _, S, M = A_x.shape
    C = A_c_kv.shape[2]
    H, D = A_w_q.shape[1], A_w_q.shape[2]
    BQ, BT, BU = 256, 256, 512
    hbm = pl.BlockSpec(memory_space=pl.ANY)
    vm = pl.BlockSpec(memory_space=pltpu.VMEM)
    V = pltpu.VMEM
    outT = pl.pallas_call(
        functools.partial(_kernel, S=S, M=M, H=H, D=D, C=C, BQ=BQ, BT=BT, BU=BU),
        out_shape=jax.ShapeDtypeStruct((M, S), F32),
        in_specs=[hbm] * 6 + [vm, vm] + [hbm] * 4 + [vm, vm, vm],
        out_specs=hbm,
        scratch_shapes=[
            V((M, S), BF16), V((S, C), BF16),
            V((2, M, D), jnp.uint32), V((2, C, D), jnp.uint32), V((2, C, D), jnp.uint32),
            V((H, M, D), BF16),
            V((M, M), BF16), V((M, M), BF16), V((M, M), BF16), V((M, M), BF16),
            V((2 * D, S), BF16), V((2, S, D), BF16), V((2 * D, S), BF16), V((H * D, S), BF16),
            V((S, M), F32), V((S, M), F32), V((BT, M), F32), V((BT, M), F32),
            V((8, 8, M), F32), V((2, M, BT), F32),
            pltpu.SemaphoreType.DMA((6,)), pltpu.SemaphoreType.DMA((S // BU,)), pltpu.SemaphoreType.DMA((3, 2)), pltpu.SemaphoreType.DMA((2,)),
        ],
        compiler_params=pltpu.CompilerParams(vmem_limit_bytes=110*1024*1024, flags={"XLA_TPU_FORCE_LP_LLO_SCHEDULER": True}),
    )(A_x[0].T, A_c_kv[0], A_w_q, A_w_uk, A_w_uv, A_w_o.transpose(0, 2, 1),
      B_Lambda_re, B_Lambda_im, B_B_re, B_B_im, B_C_re, B_C_im, B_log_dt, B_Dskip, gate_w)
    return outT.T[None]
```

```python
import functools
import math

import jax
import jax.numpy as jnp
import jax.experimental.pallas as pl
import jax.experimental.pallas.tpu as pltpu

F32 = jnp.float32
BF16 = jnp.bfloat16
NN = (((1,), (0,)), ((), ()))
NT = (((1,), (1,)), ((), ()))


def _dot(a, b, dims=NN):
    return jax.lax.dot_general(a, b, dims, preferred_element_type=F32)


def _unpack(u):
    lo = pltpu.bitcast(u << 16, F32).astype(BF16)
    hi = pltpu.bitcast(u & jnp.uint32(0xFFFF0000), F32).astype(BF16)
    return lo, hi


def _cmul(ar, ai, br, bi):
    return ar * br - ai * bi, ar * bi + ai * br


def _kernel(xT_hbm, ckv_hbm, wq_hbm, wuk_hbm, wuv_hbm, woT_hbm,
            lre_ref, lim_ref, bre_hbm, bim_hbm, cre_hbm, cim_hbm, ldt_ref, dsk_ref, gw_ref,
            out_hbm,
            xT, ckv, wq32, wkv32, woT, bre, bim, cre, cim,
            qT, kk, vT, ctxT, ur, ui, hr, hi_, coef, obuf, asum, bsum,
            sem_in, sem_x, sem_w, sem_out, *, S, M, H, D, C, BQ, BT, BU, BK):
    NP = H // 2
    wq_u = wq_hbm.bitcast(jnp.uint32)
    wuk_u = wuk_hbm.bitcast(jnp.uint32)
    wuv_u = wuv_hbm.bitcast(jnp.uint32)

    def w_copies(j, slot):
        return (pltpu.make_async_copy(wq_u.at[:, j, :], wq32.at[slot], sem_w.at[0, slot]),
                pltpu.make_async_copy(wuk_u.at[:, j, :], wkv32.at[0, slot], sem_w.at[1, slot]),
                pltpu.make_async_copy(wuv_u.at[:, j, :], wkv32.at[1, slot], sem_w.at[2, slot]))

    def x_copy(i):
        c = pl.ds(pl.multiple_of(i * BU, BU), BU)
        return pltpu.make_async_copy(xT_hbm.at[:, c], xT.at[:, c], sem_x.at[i])

    cp_c, cp_br, cp_bi, *late = [pltpu.make_async_copy(s, d, sem_in.at[i]) for i, (s, d) in enumerate(
        [(ckv_hbm, ckv), (bre_hbm, bre), (bim_hbm, bim), (woT_hbm, woT), (cre_hbm, cre), (cim_hbm, cim)])]

    cp_br.start()
    cp_bi.start()
    x_copy(0).start()

    lre = lre_ref[...].astype(F32).reshape(1, M)
    lim = lim_ref[...].astype(F32).reshape(1, M)
    dt = jnp.exp(ldt_ref[...].astype(F32)).astype(BF16).astype(F32).reshape(1, M)
    mag = jnp.exp(dt * lre)
    ar, ai = mag * jnp.cos(dt * lim), mag * jnp.sin(dt * lim)
    den = lre * lre + lim * lim
    zr, zi = _cmul(ar - 1.0, ai, lre / den, -lim / den)
    p1 = (ar, ai)
    p2 = _cmul(*p1, *p1)
    p4 = _cmul(*p2, *p2)
    rid = jax.lax.broadcasted_iota(jnp.int32, (8, M), 0)
    for n, (k, (pr, pi)) in enumerate(((1, p1), (2, p2), (4, p4))):
        coef[2 * n] = jnp.where(rid >= k, pr, 0.0)
        coef[2 * n + 1] = jnp.where(rid >= k, pi, 0.0)
    coef[6] = jnp.where(rid == 0, ar, 0.0)
    coef[7] = jnp.where(rid == 0, ai, 0.0)

    cp_br.wait()
    cp_bi.wait()
    for i in range(1, S // BU):
        x_copy(i).start()
    cp_c.start()
    for c in w_copies(0, 0):
        c.start()

    def bu_body(i, carry):
        c = pl.ds(pl.multiple_of(i * BU, BU), BU)
        x_copy(i).wait()
        x = xT[:, c].T
        a, b = _cmul(_dot(x, bre[...], NT), _dot(x, bim[...], NT), 2.0 * zr, 2.0 * zi)
        ur[c, :] = a
        ui[c, :] = b
        return carry

    jax.lax.fori_loop(0, S // BU, bu_body, 0)
    cp_c.wait()

    S2, C2 = S // 2, C // 2

    def asum_body(i, carry):
        t = pl.ds(pl.multiple_of(i * 64, 64), 64)
        u = pl.ds(pl.multiple_of(S2 + i * 64, 64), 64)
        a11, a12 = ckv[t, :C2].astype(F32), ckv[t, C2:].astype(F32)
        a21, a22 = ckv[u, :C2].astype(F32), ckv[u, C2:].astype(F32)
        for n, v in enumerate((a11 + a22, a21 + a22, a11 + a12, a21 - a11, a12 - a22)):
            asum[n, t, :] = v.astype(BF16)
        return carry

    jax.lax.fori_loop(0, S2 // 64, asum_body, 0)

    scale = (D ** -0.5) * math.log2(math.e)
    neg = -1e30

    def make_bsum(n, slot, r0=0, nr=C2, zero=jnp.uint32(0)):
        u1, u2 = wkv32[n, slot, r0:r0 + nr, :], wkv32[n, slot, C2 + r0:C2 + r0 + nr, :]
        msk, sh = jnp.uint32(0xFFFF0000) + zero, jnp.uint32(16) + zero
        b11, b21 = pltpu.bitcast(u1 << sh, F32), pltpu.bitcast(u2 << sh, F32)
        b12, b22 = pltpu.bitcast(u1 & msk, F32), pltpu.bitcast(u2 & msk, F32)
        for m, v in enumerate((b11 + b22, b11, b12 - b22, b21 - b11, b22, b11 + b12, b21 + b22)):
            bsum[m, r0:r0 + nr, pl.ds(pl.multiple_of(n * D, D), D)] = v.astype(BF16)

    for c in w_copies(0, 0):
        c.wait()
    jax.lax.fori_loop(0, 2, lambda n, c: make_bsum(n, 0), None)

    def pair_body(j, carry):
        slot = j % 2

        @pl.when(j + 1 < NP)
        def _():
            for c in w_copies(j + 1, 1 - slot):
                c.start()

        @pl.when(j == 0)
        def _():
            for c in late:
                c.start()

        lo, hi = _unpack(wq32[slot].T)
        wqT = jnp.concatenate([lo, hi], axis=0)
        qT[...] = (_dot(wqT, xT[...]) * scale).astype(BF16)

        def kv_body(i, carry2):
            t = pl.ds(pl.multiple_of(i * BK, BK), BK)
            u = pl.ds(pl.multiple_of(S2 + i * BK, BK), BK)

            def put(e, rows, val):
                val = val.astype(BF16)
                kk[e, rows, :] = val[:, :D]
                vT[e * D:(e + 1) * D, rows] = val[:, D:].T

            m2 = _dot(asum[1, t, :], bsum[1])
            m4 = _dot(ckv[u, C2:], bsum[3])
            put(0, u, m2 + m4)
            m5 = _dot(asum[2, t, :], bsum[4])
            m3 = _dot(ckv[t, :C2], bsum[2])
            put(1, t, m3 + m5)
            d1, d2 = m4 - m5, m3 - m2
            m1 = _dot(asum[0, t, :], bsum[0])
            d1, d2 = d1 + m1, d2 + m1
            put(0, t, d1 + _dot(asum[4, t, :], bsum[6]))
            put(1, u, d2 + _dot(asum[3, t, :], bsum[5]))
            return carry2

        jax.lax.fori_loop(0, S2 // BK, kv_body, 0)

        @pl.when(j + 1 < NP)
        def _():
            for c in w_copies(j + 1, 1 - slot):
                c.wait()

        def head_body(e, carry2):
            r = pl.ds(pl.multiple_of(e * D, D), D)
            ro = pl.ds(pl.multiple_of((2 * j + e) * D, D), D)
            nq = S // BQ
            T = BQ // 2
            row = jax.lax.broadcasted_iota(jnp.int32, (T, T), 0)
            col = jax.lax.broadcasted_iota(jnp.int32, (T, T), 1)
            tri = row <= col

            def scores(i):
                L = i * BQ + T
                q = qT[r, i * BQ:(i + 1) * BQ]
                s = _dot(kk[e, 0:L, :], q)
                sx = jnp.where(tri, _dot(kk[e, L:L + T, :], q[:, T:]), neg)
                sd = jnp.concatenate([jnp.where(tri, s[L - T:, :T], neg), s[L - T:, T:]], axis=1)
                if i > 0:
                    sd = jnp.concatenate([s[:L - T], sd], axis=0)
                m = jnp.max(sd, axis=0, keepdims=True)
                m = jnp.concatenate([m[:, :T], jnp.maximum(m[:, T:], jnp.max(sx, axis=0, keepdims=True))], axis=1)
                return sd, sx, m

            nxt = scores(0)
            for i in range(nq):
                s, sx, m = nxt
                if i + 1 < nq:
                    nxt = scores(i + 1)
                L = i * BQ + T
                p = jnp.exp2(s - m)
                px = jnp.exp2(sx - m[:, T:])
                l = jnp.sum(p, axis=0, keepdims=True)
                o = _dot(vT[r, 0:L], p.astype(BF16))
                ox = _dot(vT[r, L:L + T], px.astype(BF16))
                la = 1.0 / l[:, :T]
                lb = 1.0 / (l[:, T:] + jnp.sum(px, axis=0, keepdims=True))
                ctxT[ro, i * BQ:L] = (o[:, :T] * la).astype(BF16)
                ctxT[ro, L:L + T] = ((o[:, T:] + ox) * lb).astype(BF16)
                for c in range(i + 1):
                    n = i * (i + 1) // 2 + c - 4
                    if n >= 0:
                        make_bsum(e, 1 - slot, n * 16, 16, (s[c * BQ:c * BQ + 16] < 2 * neg).astype(jnp.uint32))
            return carry2

        jax.lax.fori_loop(0, 2, head_body, 0)
        return carry

    jax.lax.fori_loop(0, NP, pair_body, 0)

    for c in late:
        c.wait()

    gcol = jnp.broadcast_to(gw_ref[...].astype(F32).reshape(1, M), (128, M)).T
    dcol = jnp.broadcast_to(dsk_ref[...].astype(F32).reshape(1, M), (128, M)).T

    def out_copy(i, slot):
        return pltpu.make_async_copy(
            obuf.at[slot], out_hbm.at[:, pl.ds(pl.multiple_of(i * BT, BT), BT)], sem_out.at[slot])

    def out_body(i, carry):
        car, cai = carry
        c = pl.ds(pl.multiple_of(i * BT, BT), BT)
        slot = i % 2
        bx = xT[:, c]
        for g in range(BT // 8):
            t = pl.ds(pl.multiple_of(i * BT + g * 8, 8), 8)
            dr, di = _cmul(coef[6], coef[7], pltpu.roll(car, 1, 0), pltpu.roll(cai, 1, 0))
            a, b = ur[t, :] + dr, ui[t, :] + di
            for n, k in enumerate((1, 2, 4)):
                dr, di = _cmul(coef[2 * n], coef[2 * n + 1], pltpu.roll(a, k, 0), pltpu.roll(b, k, 0))
                a, b = a + dr, b + di
            car, cai = a, b
            hr[g * 8:(g + 1) * 8, :] = a
            hi_[g * 8:(g + 1) * 8, :] = b
        att = _dot(woT[0], ctxT[0:D, c])
        for h in range(1, H):
            att = att + _dot(woT[h], ctxT[h * D:(h + 1) * D, c])
        y = _dot(cre[...], hr[...].astype(BF16), NT) - _dot(cim[...], hi_[...].astype(BF16), NT)
        rep = BT // 128
        y = y + bx.astype(F32) * jnp.tile(dcol, (1, rep))
        z = jnp.sum(bx.astype(F32) * jnp.tile(gcol, (1, rep)), axis=0, keepdims=True)
        gate = 1.0 / (1.0 + jnp.exp(-z))

        @pl.when(i >= 2)
        def _():
            out_copy(i - 2, slot).wait()

        obuf[slot] = gate * att + (1.0 - gate) * y
        out_copy(i, slot).start()
        return car, cai

    zero = jnp.zeros((8, M), F32)
    nb = S // BT
    jax.lax.fori_loop(0, nb, out_body, (zero, zero))
    out_copy(nb - 2, (nb - 2) % 2).wait()
    out_copy(nb - 1, (nb - 1) % 2).wait()


@jax.jit
def pallas_gated_mix__compressed_kv_cla__ssm_conv_s5__prompt_kernel(
    A_x, A_c_kv, A_w_q, A_w_uk, A_w_uv, A_w_o, B_x, B_Lambda_re, B_Lambda_im,
    B_B_re, B_B_im, B_C_re, B_C_im, B_log_dt, B_Dskip, gate_w,
):
    _, S, M = A_x.shape
    C = A_c_kv.shape[2]
    H, D = A_w_q.shape[1], A_w_q.shape[2]
    BQ, BT, BU, BK = 256, 256, 512, 1024
    hbm = pl.BlockSpec(memory_space=pl.ANY)
    vm = pl.BlockSpec(memory_space=pltpu.VMEM)
    V = pltpu.VMEM
    outT = pl.pallas_call(
        functools.partial(_kernel, S=S, M=M, H=H, D=D, C=C, BQ=BQ, BT=BT, BU=BU, BK=BK),
        out_shape=jax.ShapeDtypeStruct((M, S), F32),
        in_specs=[hbm] * 6 + [vm, vm] + [hbm] * 4 + [vm, vm, vm],
        out_specs=hbm,
        scratch_shapes=[
            V((M, S), BF16), V((S, C), BF16),
            V((2, M, D), jnp.uint32), V((2, 2, C, D), jnp.uint32),
            V((H, M, D), BF16),
            V((M, M), BF16), V((M, M), BF16), V((M, M), BF16), V((M, M), BF16),
            V((2 * D, S), BF16), V((2, S, D), BF16), V((2 * D, S), BF16), V((H * D, S), BF16),
            V((S, M), F32), V((S, M), F32), V((BT, M), F32), V((BT, M), F32),
            V((8, 8, M), F32), V((2, M, BT), F32), V((5, S // 2, C // 2), BF16), V((7, C // 2, 2 * D), BF16),
            pltpu.SemaphoreType.DMA((6,)), pltpu.SemaphoreType.DMA((S // BU,)), pltpu.SemaphoreType.DMA((3, 2)), pltpu.SemaphoreType.DMA((2,)),
        ],
        compiler_params=pltpu.CompilerParams(vmem_limit_bytes=110*1024*1024, flags={"XLA_TPU_FORCE_LP_LLO_SCHEDULER": True}),
    )(A_x[0].T, A_c_kv[0], A_w_q, A_w_uk, A_w_uv, A_w_o.transpose(0, 2, 1),
      B_Lambda_re, B_Lambda_im, B_B_re, B_B_im, B_C_re, B_C_im, B_log_dt, B_Dskip, gate_w)
    return outT.T[None]
```

```python
import functools
import math

import jax
import jax.numpy as jnp
import jax.experimental.pallas as pl
import jax.experimental.pallas.tpu as pltpu

F32 = jnp.float32
BF16 = jnp.bfloat16
NN = (((1,), (0,)), ((), ()))
NT = (((1,), (1,)), ((), ()))


def _dot(a, b, dims=NN):
    return jax.lax.dot_general(a, b, dims, preferred_element_type=F32)


def _unpack(u):
    lo = pltpu.bitcast(u << 16, F32).astype(BF16)
    hi = pltpu.bitcast(u & jnp.uint32(0xFFFF0000), F32).astype(BF16)
    return lo, hi


def _cmul(ar, ai, br, bi):
    return ar * br - ai * bi, ar * bi + ai * br


def _kernel(xT_hbm, ckv_hbm, wq_hbm, wuk_hbm, wuv_hbm, woT_hbm,
            lre_ref, lim_ref, bre_hbm, bim_hbm, cre_hbm, cim_hbm, ldt_ref, dsk_ref, gw_ref,
            out_hbm,
            xT, ckv, wq32, wkv32, woT, bre, bim, cre, cim,
            qT, kk, vT, ctxT, ur, ui, hr, hi_, coef, obuf, asum, bsum,
            sem_in, sem_x, sem_w, sem_out, *, S, M, H, D, C, BQ, BT, BU, BK):
    NP = H // 2
    wq_u = wq_hbm.bitcast(jnp.uint32)
    wuk_u = wuk_hbm.bitcast(jnp.uint32)
    wuv_u = wuv_hbm.bitcast(jnp.uint32)

    def w_copies(j, slot):
        return (pltpu.make_async_copy(wq_u.at[:, j, :], wq32.at[slot], sem_w.at[0, slot]),
                pltpu.make_async_copy(wuk_u.at[:, j, :], wkv32.at[0, slot], sem_w.at[1, slot]),
                pltpu.make_async_copy(wuv_u.at[:, j, :], wkv32.at[1, slot], sem_w.at[2, slot]))

    def x_copy(i):
        c = pl.ds(pl.multiple_of(i * BU, BU), BU)
        return pltpu.make_async_copy(xT_hbm.at[:, c], xT.at[:, c], sem_x.at[i])

    cp_c, cp_br, cp_bi, *late = [pltpu.make_async_copy(s, d, sem_in.at[i]) for i, (s, d) in enumerate(
        [(ckv_hbm, ckv), (bre_hbm, bre), (bim_hbm, bim), (woT_hbm, woT), (cre_hbm, cre), (cim_hbm, cim)])]

    cp_br.start()
    cp_bi.start()
    x_copy(0).start()

    lre = lre_ref[...].astype(F32).reshape(1, M)
    lim = lim_ref[...].astype(F32).reshape(1, M)
    dt = jnp.exp(ldt_ref[...].astype(F32)).astype(BF16).astype(F32).reshape(1, M)
    mag = jnp.exp(dt * lre)
    ar, ai = mag * jnp.cos(dt * lim), mag * jnp.sin(dt * lim)
    den = lre * lre + lim * lim
    zr, zi = _cmul(ar - 1.0, ai, lre / den, -lim / den)
    p1 = (ar, ai)
    p2 = _cmul(*p1, *p1)
    p4 = _cmul(*p2, *p2)
    rid = jax.lax.broadcasted_iota(jnp.int32, (8, M), 0)
    for n, (k, (pr, pi)) in enumerate(((1, p1), (2, p2), (4, p4))):
        coef[2 * n] = jnp.where(rid >= k, pr, 0.0)
        coef[2 * n + 1] = jnp.where(rid >= k, pi, 0.0)
    coef[6] = jnp.where(rid == 0, ar, 0.0)
    coef[7] = jnp.where(rid == 0, ai, 0.0)

    cp_br.wait()
    cp_bi.wait()
    for i in range(1, S // BU):
        x_copy(i).start()
    cp_c.start()
    for c in w_copies(0, 0):
        c.start()

    def bu_body(i, carry):
        c = pl.ds(pl.multiple_of(i * BU, BU), BU)
        x_copy(i).wait()
        x = xT[:, c].T
        a, b = _cmul(_dot(x, bre[...], NT), _dot(x, bim[...], NT), 2.0 * zr, 2.0 * zi)
        ur[c, :] = a
        ui[c, :] = b
        return carry

    jax.lax.fori_loop(0, S // BU, bu_body, 0)
    cp_c.wait()

    S2, C2 = S // 2, C // 2

    def asum_body(i, carry):
        t = pl.ds(pl.multiple_of(i * 32, 32), 32)
        u = pl.ds(pl.multiple_of(S2 + i * 32, 32), 32)
        a11, a12 = ckv[t, :C2].astype(F32), ckv[t, C2:].astype(F32)
        a21, a22 = ckv[u, :C2].astype(F32), ckv[u, C2:].astype(F32)
        for n, v in enumerate((a11 + a22, a21 + a22, a11 + a12, a21 - a11, a12 - a22)):
            asum[n, t, :] = v.astype(BF16)
        return carry

    jax.lax.fori_loop(0, S2 // 32, asum_body, 0)

    scale = (D ** -0.5) * math.log2(math.e)
    neg = -1e30

    def make_bsum(n, slot, r0, nr=16, zero=jnp.uint32(0)):
        u1, u2 = wkv32[n, slot, pl.ds(r0, nr), :], wkv32[n, slot, pl.ds(C2 + r0, nr), :]
        msk, sh = jnp.uint32(0xFFFF0000) + zero, jnp.uint32(16) + zero
        b11, b21 = pltpu.bitcast(u1 << sh, F32), pltpu.bitcast(u2 << sh, F32)
        b12, b22 = pltpu.bitcast(u1 & msk, F32), pltpu.bitcast(u2 & msk, F32)
        for m, v in enumerate((b11 + b22, b11, b12 - b22, b21 - b11, b22, b11 + b12, b21 + b22)):
            bsum[m, pl.ds(r0, nr), pl.ds(n * D if isinstance(n, int) else pl.multiple_of(n * D, D), D)] = v.astype(BF16)

    for c in w_copies(0, 0):
        c.wait()

    def bsum0_body(i, carry):
        for n in range(2):
            make_bsum(n, 0, pl.multiple_of(i * 32, 32), 32)
        return carry

    jax.lax.fori_loop(0, C2 // 32, bsum0_body, 0)

    def pair_body(j, carry):
        slot = j % 2

        @pl.when(j + 1 < NP)
        def _():
            for c in w_copies(j + 1, 1 - slot):
                c.start()

        @pl.when(j == 0)
        def _():
            for c in late:
                c.start()

        lo, hi = _unpack(wq32[slot].T)
        wqT = jnp.concatenate([lo, hi], axis=0)
        qT[...] = (_dot(wqT, xT[...]) * scale).astype(BF16)

        def kv_body(i, carry2):
            t = pl.ds(pl.multiple_of(i * BK, BK), BK)
            u = pl.ds(pl.multiple_of(S2 + i * BK, BK), BK)

            def put(e, rows, val):
                val = val.astype(BF16)
                kk[e, rows, :] = val[:, :D]
                vT[e * D:(e + 1) * D, rows] = val[:, D:].T

            m2 = _dot(asum[1, t, :], bsum[1])
            m4 = _dot(ckv[u, C2:], bsum[3])
            put(0, u, m2 + m4)
            m5 = _dot(asum[2, t, :], bsum[4])
            m3 = _dot(ckv[t, :C2], bsum[2])
            put(1, t, m3 + m5)
            d1, d2 = m4 - m5, m3 - m2
            m1 = _dot(asum[0, t, :], bsum[0])
            d1, d2 = d1 + m1, d2 + m1
            put(0, t, d1 + _dot(asum[4, t, :], bsum[6]))
            put(1, u, d2 + _dot(asum[3, t, :], bsum[5]))
            return carry2

        jax.lax.fori_loop(0, S2 // BK, kv_body, 0)

        @pl.when(j + 1 < NP)
        def _():
            for c in w_copies(j + 1, 1 - slot):
                c.wait()

        def head_body(e, carry2):
            r = pl.ds(pl.multiple_of(e * D, D), D)
            ro = pl.ds(pl.multiple_of((2 * j + e) * D, D), D)
            nq = S // BQ
            T = BQ // 2
            row = jax.lax.broadcasted_iota(jnp.int32, (T, T), 0)
            col = jax.lax.broadcasted_iota(jnp.int32, (T, T), 1)
            tri = row <= col

            def scores(i):
                L = i * BQ + T
                q = qT[r, i * BQ:(i + 1) * BQ]
                s = _dot(kk[e, 0:L, :], q)
                sx = jnp.where(tri, _dot(kk[e, L:L + T, :], q[:, T:]), neg)
                sd = jnp.concatenate([jnp.where(tri, s[L - T:, :T], neg), s[L - T:, T:]], axis=1)
                if i > 0:
                    sd = jnp.concatenate([s[:L - T], sd], axis=0)
                m = jnp.max(sd, axis=0, keepdims=True)
                m = jnp.concatenate([m[:, :T], jnp.maximum(m[:, T:], jnp.max(sx, axis=0, keepdims=True))], axis=1)
                return sd, sx, m

            nxt = scores(0)
            for i in range(nq):
                s, sx, m = nxt
                if i + 1 < nq:
                    nxt = scores(i + 1)
                L = i * BQ + T
                p = jnp.exp2(s - m)
                px = jnp.exp2(sx - m[:, T:])
                l = jnp.sum(p, axis=0, keepdims=True)
                o = _dot(vT[r, 0:L], p.astype(BF16))
                ox = _dot(vT[r, L:L + T], px.astype(BF16))
                la = 1.0 / l[:, :T]
                lb = 1.0 / (l[:, T:] + jnp.sum(px, axis=0, keepdims=True))
                ctxT[ro, i * BQ:L] = (o[:, :T] * la).astype(BF16)
                ctxT[ro, L:L + T] = ((o[:, T:] + ox) * lb).astype(BF16)
                for c in range(i + 1):
                    n = i * (i + 1) // 2 + c - 4
                    if n >= 0:
                        make_bsum(e, 1 - slot, n * 16, 16, (s[c * BQ:c * BQ + 16] < 2 * neg).astype(jnp.uint32))
            return carry2

        jax.lax.fori_loop(0, 2, head_body, 0)
        return carry

    jax.lax.fori_loop(0, NP, pair_body, 0)

    for c in late:
        c.wait()

    gcol = jnp.broadcast_to(gw_ref[...].astype(F32).reshape(1, M), (128, M)).T
    dcol = jnp.broadcast_to(dsk_ref[...].astype(F32).reshape(1, M), (128, M)).T

    def out_copy(i, slot):
        return pltpu.make_async_copy(
            obuf.at[slot], out_hbm.at[:, pl.ds(pl.multiple_of(i * BT, BT), BT)], sem_out.at[slot])

    def out_body(i, carry):
        car, cai = carry
        c = pl.ds(pl.multiple_of(i * BT, BT), BT)
        slot = i % 2
        bx = xT[:, c]
        att = _dot(woT[0], ctxT[0:D, c])
        parts = [att]
        for h in range(1, H):
            att = att + _dot(woT[h], ctxT[h * D:(h + 1) * D, c])
            parts.append(att)
        for g in range(BT // 8):
            t = pl.ds(pl.multiple_of(i * BT + g * 8, 8), 8)
            dr, di = _cmul(coef[6], coef[7], pltpu.roll(car, 1, 0), pltpu.roll(cai, 1, 0))
            w = pltpu.bitcast(parts[g // 4][(g % 4) * 112:(g % 4) * 112 + 8, :128], jnp.int32)
            z = jnp.tile((jnp.abs(w >> 1) >> 31), (1, 4))[:, :M]
            a, b = pltpu.bitcast(pltpu.bitcast(ur[t, :], jnp.int32) | z, F32) + dr, ui[t, :] + di
            for n, k in enumerate((1, 2, 4)):
                dr, di = _cmul(coef[2 * n], coef[2 * n + 1], pltpu.roll(a, k, 0), pltpu.roll(b, k, 0))
                a, b = a + dr, b + di
            car, cai = a, b
            hr[g * 8:(g + 1) * 8, :] = a
            hi_[g * 8:(g + 1) * 8, :] = b
        y = _dot(cre[...], hr[...].astype(BF16), NT) - _dot(cim[...], hi_[...].astype(BF16), NT)
        rep = BT // 128
        y = y + bx.astype(F32) * jnp.tile(dcol, (1, rep))
        z = jnp.sum(bx.astype(F32) * jnp.tile(gcol, (1, rep)), axis=0, keepdims=True)
        gate = 1.0 / (1.0 + jnp.exp(-z))

        @pl.when(i >= 2)
        def _():
            out_copy(i - 2, slot).wait()

        obuf[slot] = gate * att + (1.0 - gate) * y
        out_copy(i, slot).start()
        return car, cai

    zero = jnp.zeros((8, M), F32)
    nb = S // BT
    jax.lax.fori_loop(0, nb, out_body, (zero, zero))
    out_copy(nb - 2, (nb - 2) % 2).wait()
    out_copy(nb - 1, (nb - 1) % 2).wait()


@jax.jit
def pallas_gated_mix__compressed_kv_cla__ssm_conv_s5__prompt_kernel(
    A_x, A_c_kv, A_w_q, A_w_uk, A_w_uv, A_w_o, B_x, B_Lambda_re, B_Lambda_im,
    B_B_re, B_B_im, B_C_re, B_C_im, B_log_dt, B_Dskip, gate_w,
):
    _, S, M = A_x.shape
    C = A_c_kv.shape[2]
    H, D = A_w_q.shape[1], A_w_q.shape[2]
    BQ, BT, BU, BK = 256, 256, 512, 1024
    hbm = pl.BlockSpec(memory_space=pl.ANY)
    vm = pl.BlockSpec(memory_space=pltpu.VMEM)
    V = pltpu.VMEM
    outT = pl.pallas_call(
        functools.partial(_kernel, S=S, M=M, H=H, D=D, C=C, BQ=BQ, BT=BT, BU=BU, BK=BK),
        out_shape=jax.ShapeDtypeStruct((M, S), F32),
        in_specs=[hbm] * 6 + [vm, vm] + [hbm] * 4 + [vm, vm, vm],
        out_specs=hbm,
        scratch_shapes=[
            V((M, S), BF16), V((S, C), BF16),
            V((2, M, D), jnp.uint32), V((2, 2, C, D), jnp.uint32),
            V((H, M, D), BF16),
            V((M, M), BF16), V((M, M), BF16), V((M, M), BF16), V((M, M), BF16),
            V((2 * D, S), BF16), V((2, S, D), BF16), V((2 * D, S), BF16), V((H * D, S), BF16),
            V((S, M), F32), V((S, M), F32), V((BT, M), F32), V((BT, M), F32),
            V((8, 8, M), F32), V((2, M, BT), F32), V((5, S // 2, C // 2), BF16), V((7, C // 2, 2 * D), BF16),
            pltpu.SemaphoreType.DMA((6,)), pltpu.SemaphoreType.DMA((S // BU,)), pltpu.SemaphoreType.DMA((3, 2)), pltpu.SemaphoreType.DMA((2,)),
        ],
        compiler_params=pltpu.CompilerParams(vmem_limit_bytes=110*1024*1024, flags={"XLA_TPU_FORCE_LP_LLO_SCHEDULER": True}),
    )(A_x[0].T, A_c_kv[0], A_w_q, A_w_uk, A_w_uv, A_w_o.transpose(0, 2, 1),
      B_Lambda_re, B_Lambda_im, B_B_re, B_B_im, B_C_re, B_C_im, B_log_dt, B_Dskip, gate_w)
    return outT.T[None]
```
